```python
import os as _os
_os.environ.setdefault("JAX_PLATFORMS", "cpu")
import jax
import jax.numpy as jnp

def _softmax(x, axis=-1):
    return jax.nn.softmax(x, axis=axis)
def _gelu(x):
    return jax.nn.gelu(x, approximate=True)
def _silu(x):
    return jax.nn.silu(x)
def _sigmoid(x):
    return jax.nn.sigmoid(x)
def _layernorm(x, axis=-1, eps=1e-5):
    m = jnp.mean(x, axis=axis, keepdims=True)
    v = jnp.var(x, axis=axis, keepdims=True)
    return (x - m) / jnp.sqrt(v + eps)
def _scatter_add(tgt, idx, src, axis=0):
    return tgt.at[idx].add(src)
def _segment_sum(src, seg, n):
    return jax.ops.segment_sum(src, seg, n)
class _Rng:
    def __init__(self, key):
        self._k = key
    def _next(self):
        self._k, sub = jax.random.split(self._k)
        return sub
    def normal(self, shape):
        return jax.random.normal(self._next(), shape, dtype=jnp.bfloat16)
    def randint(self, lo, hi, shape):
        return jax.random.randint(self._next(), shape, lo, hi, dtype=jnp.int32)
    def uniform(self, shape, lo=0.0, hi=1.0):
        return jax.random.uniform(self._next(), shape, jnp.bfloat16, lo, hi)
    def permutation(self, n):
        return jax.random.permutation(self._next(), n)


kernel_name = 'sequential_preLN__softmax_full_mha__glu_gated_swiglu__prompt'

def setup_inputs():
    _rng = _Rng(jax.random.key(int.from_bytes(__import__("os").urandom(4), "little")))
    _w = (lambda a: (lambda t: t.astype(jnp.bfloat16) if jnp.issubdtype(t.dtype, jnp.floating) else t)(jnp.asarray(a)))
    def _A_setup():
        B, S, D = 1, 2048, 640
        return {
            "x": _w((lambda *s: _rng.normal(s) * 0.05)(B, S, D)),
            "wqkv": _w((lambda *s: _rng.normal(s) * 0.05)(D, 3 * D)),
            "wo": _w((lambda *s: _rng.normal(s) * 0.05)(D, D)),
        }
    _A_in = _A_setup()

    def _B_setup():
        B, S, D, F = 1, 2048, 640, 1728
        return {
            "x": _w((lambda *s: _rng.normal(s) * 0.05)(B, S, D)),
            "w1": _w((lambda *s: _rng.normal(s) * 0.05)(D, F) * (2.0 / D) ** 0.5),
            "w3": _w((lambda *s: _rng.normal(s) * 0.05)(D, F) * (2.0 / D) ** 0.5),
            "w2": _w((lambda *s: _rng.normal(s) * 0.05)(F, D) * (2.0 / F) ** 0.5),
        }
    _B_in = _B_setup()

    return {
        "A_x": _A_in["x"],
        "A_wqkv": _A_in["wqkv"],
        "A_wo": _A_in["wo"],
        "B_x": _B_in["x"],
        "B_w1": _B_in["w1"],
        "B_w3": _B_in["w3"],
        "B_w2": _B_in["w2"],
    }

def reference(A_x, A_wqkv, A_wo, B_x, B_w1, B_w3, B_w2):
    def _A_ref(x, wqkv, wo):
        B, S, D = x.shape
        H = 32; Dh = D // H
        qkv = (lambda x, *d: x.transpose(*d))((x @ wqkv).reshape(B, S, 3, H, Dh), 2, 0, 3, 1, 4)
        q, k, v = qkv[0], qkv[1], qkv[2]
        scale = Dh ** -0.5
        scores = jnp.einsum("bhqd,bhkd->bhqk", q, k) * scale
        p = _softmax(scores, axis=-1)
        o = jnp.einsum("bhqk,bhkd->bhqd", p, v)
        return (lambda x, *d: x.transpose(*d))(o, 0, 2, 1, 3).reshape(B, S, D) @ wo

    def _B_ref(x, w1, w3, w2):
        gate = jnp.einsum("bsd,df->bsf", x, w1)
        up = jnp.einsum("bsd,df->bsf", x, w3)
        h = _silu(gate) * up
        out = jnp.einsum("bsf,fd->bsd", h, w2)
        return out

    x = A_x
    h = x + _A_ref(_layernorm(x, axis=-1), A_wqkv, A_wo)
    h2 = h + _B_ref(_layernorm(h, axis=-1), B_w1, B_w3, B_w2)
    return h2
```

```python
import functools

import jax
import jax.numpy as jnp
import jax.experimental.pallas as pl
import jax.experimental.pallas.tpu as pltpu

_EPS = 1e-5
_LOG2E = 1.4426950408889634


def _ln(x):
    m = jnp.mean(x, axis=-1, keepdims=True)
    xc = x - m
    v = jnp.mean(xc * xc, axis=-1, keepdims=True)
    return xc * jax.lax.rsqrt(v + _EPS)


def _kernel(x_ref, wqkv_ref, wo_hbm, w1t_hbm, w3t_hbm, w2_hbm, o_ref,
            wo_ref, w1t_ref, w3t_ref, w2_ref, sems,
            k_scr, qt_scr, vt_scr, wo_scr, ot_scr, sa_scr, sb_scr,
            *, S, D, H, Dh, F, TQ, R):
    G = 128 // Dh
    DP = k_scr.shape[1]
    VR = vt_scr.shape[0] // H
    f32, bf16 = jnp.float32, jnp.bfloat16

    copies = [pltpu.make_async_copy(src, dst, sems.at[i])
              for i, (src, dst) in enumerate(((wo_hbm, wo_ref), (w1t_hbm, w1t_ref),
                                              (w3t_hbm, w3t_ref), (w2_hbm, w2_ref)))]
    for cp in copies:
        cp.start()

    with jax.named_scope('phase0'):
        xn = _ln(x_ref[...].astype(f32)).astype(bf16)
        c = jax.lax.broadcasted_iota(jnp.int32, (D, DP), 0)
        j = jax.lax.broadcasted_iota(jnp.int32, (D, DP), 1)
        hh = c // Dh
        pqk = (j == (hh // G) * 128 + (hh % G) * Dh + c % Dh).astype(bf16)
        wk = jnp.dot(wqkv_ref[:, D:2 * D], pqk, preferred_element_type=f32).astype(bf16)
        k_scr[...] = jnp.dot(xn, wk, preferred_element_type=f32).astype(bf16)

        tn = (((0,), (1,)), ((), ()))
        qt = jax.lax.dot_general(wqkv_ref[:, 0:D], xn, tn, preferred_element_type=f32)
        qt = qt * (Dh ** -0.5 * _LOG2E)
        vt = jax.lax.dot_general(wqkv_ref[:, 2 * D:3 * D], xn, tn,
                                 preferred_element_type=f32)
        qt_scr[...] = jnp.zeros_like(qt_scr)
        r = jax.lax.broadcasted_iota(jnp.int32, (H * VR, S), 0)
        vt_scr[...] = jnp.where(r % VR == Dh, 1.0, 0.0).astype(bf16)
        for h in range(H):
            q_lo = (h // G) * 128 + (h % G) * Dh
            qt_scr[q_lo:q_lo + Dh, :] = qt[h * Dh:(h + 1) * Dh, :].astype(bf16)
            vt_scr[h * VR:h * VR + Dh, :] = vt[h * Dh:(h + 1) * Dh, :].astype(bf16)

        copies[0].wait()
        wo = wo_ref[...].astype(f32)
        wo_scr[...] = jnp.zeros_like(wo_scr)
        for h in range(H):
            wo_scr[h * VR:h * VR + Dh, :] = wo[h * Dh:(h + 1) * Dh, :].astype(bf16)

    for cp in copies[1:]:
        cp.wait()

    def qtile(step, carry0):
        q0 = pl.multiple_of(step * TQ, TQ)

        def masked_q(h):
            t = h // G
            i = h % G
            lo = pl.multiple_of(t * 128, 128)
            qt = qt_scr[pl.ds(lo, 128), pl.ds(q0, TQ)]
            r = jax.lax.broadcasted_iota(jnp.int32, (128, TQ), 0)
            qm = jnp.where((r >= i * Dh) & (r < (i + 1) * Dh), qt, jnp.zeros_like(qt))
            return lo, qm

        def step(ha, sa_ref, hb, sb_ref, mb):
            if ha is not None:
                lo, qm = masked_q(ha)
                m8 = jnp.full((8, TQ), -jnp.inf, f32)
            if hb is not None:
                v0 = pl.multiple_of(hb * VR, VR)
                acc = jnp.zeros((VR, TQ), f32)
            for c in range(S // R):
                rows = pl.ds(c * R, R)
                if ha is not None:
                    sa = jnp.dot(k_scr[rows, pl.ds(lo, 128)], qm,
                                 preferred_element_type=f32)
                    sa_ref[rows, :] = sa
                    m8 = jnp.maximum(m8, jnp.max(sa.reshape(R // 8, 8, TQ), axis=0))
                if hb is not None:
                    p = jnp.exp2(sb_ref[rows, :] - mb).astype(bf16)
                    acc = acc + jnp.dot(vt_scr[pl.ds(v0, VR), rows], p,
                                        preferred_element_type=f32)
            if hb is not None:
                l = acc[Dh:Dh + 1, :]
                ot_scr[pl.ds(v0, VR), :] = (acc / l).astype(bf16)
            if ha is not None:
                return jnp.max(m8, axis=0, keepdims=True)

        def pair(j, ma):
            h0 = 2 * j
            mb = step(h0 + 1, sb_scr, h0, sa_scr, ma)
            return step(h0 + 2, sa_scr, h0 + 1, sb_scr, mb)

        with jax.named_scope('attn'):
            ma = step(0, sa_scr, None, None, None)
            ma = jax.lax.fori_loop(0, H // 2 - 1, pair, ma)
            mb = step(H - 1, sb_scr, H - 2, sa_scr, ma)
            step(None, None, H - 1, sb_scr, mb)

        with jax.named_scope('wo'):
            attn = jax.lax.dot_general(ot_scr[...], wo_scr[...], (((0,), (0,)), ((), ())),
                                       preferred_element_type=f32)
        h1 = x_ref[pl.ds(q0, TQ), :].astype(f32) + attn

        with jax.named_scope('ffn'):
            hn = _ln(h1).astype(bf16)
            nt = (((1,), (1,)), ((), ()))
            gate = jax.lax.dot_general(hn, w1t_ref[...], nt, preferred_element_type=f32)
            up = jax.lax.dot_general(hn, w3t_ref[...], nt, preferred_element_type=f32)
            act = (gate * jax.nn.sigmoid(gate) * up).astype(bf16)
            out = jnp.dot(act, w2_ref[...], preferred_element_type=f32)
        o_ref[pl.ds(q0, TQ), :] = (h1 + out).astype(o_ref.dtype)
        return carry0

    jax.lax.fori_loop(0, S // TQ, qtile, 0)


@jax.jit
def pallas_sequential_preLN__softmax_full_mha__glu_gated_swiglu__prompt_kernel(
    A_x: jax.Array,
    A_wqkv: jax.Array,
    A_wo: jax.Array,
    B_x: jax.Array,
    B_w1: jax.Array,
    B_w3: jax.Array,
    B_w2: jax.Array,
):
    B, S, D = A_x.shape
    assert B == 1
    F = B_w1.shape[1]
    H = 32
    Dh = D // H
    G = 128 // Dh
    NT = -(-H // G)
    DP = NT * 128
    VR = 32
    TQ = 512
    R = 256
    x = A_x.reshape(S, D)
    bf16 = jnp.bfloat16

    kernel = functools.partial(_kernel, S=S, D=D, H=H, Dh=Dh, F=F, TQ=TQ, R=R)
    vmem = pl.BlockSpec(memory_space=pltpu.VMEM)
    hbm = pl.BlockSpec(memory_space=pl.ANY)
    out = pl.pallas_call(
        kernel,
        out_shape=jax.ShapeDtypeStruct((S, D), A_x.dtype),
        in_specs=[vmem, vmem, hbm, hbm, hbm, hbm],
        out_specs=vmem,
        scratch_shapes=[
            pltpu.VMEM((D, D), bf16),
            pltpu.VMEM((F, D), bf16),
            pltpu.VMEM((F, D), bf16),
            pltpu.VMEM((F, D), bf16),
            pltpu.SemaphoreType.DMA((4,)),
            pltpu.VMEM((S, DP), bf16),
            pltpu.VMEM((DP, S), bf16),
            pltpu.VMEM((H * VR, S), bf16),
            pltpu.VMEM((H * VR, D), bf16),
            pltpu.VMEM((H * VR, TQ), bf16),
            pltpu.VMEM((S, TQ), jnp.float32),
            pltpu.VMEM((S, TQ), jnp.float32),
        ],
        compiler_params=pltpu.CompilerParams(
            vmem_limit_bytes=100 * 1024 * 1024,
        ),
    )(x, A_wqkv, A_wo, B_w1.T, B_w3.T, B_w2)
    return out.reshape(B, S, D)
```

```python
import functools

import jax
import jax.numpy as jnp
import jax.experimental.pallas as pl
import jax.experimental.pallas.tpu as pltpu

_EPS = 1e-5
_LOG2E = 1.4426950408889634


def _ln(x):
    m = jnp.mean(x, axis=-1, keepdims=True)
    xc = x - m
    v = jnp.mean(xc * xc, axis=-1, keepdims=True)
    return xc * jax.lax.rsqrt(v + _EPS)


def _kernel(x_ref, wqkv_ref, wo_hbm, w1t_hbm, w3t_hbm, w2_hbm, o_hbm,
            wo_ref, w1t_ref, w3t_ref, w2_ref, o_ref,
            in_sems, out_sems,
            k_scr, qt_scr, vt_scr, ot_scr, otc_scr, sa_scr, sb_scr,
            *, S, D, H, Dh, F, TQ, R):
    G = 128 // Dh
    DP = k_scr.shape[1]
    VR = vt_scr.shape[0] // H
    f32, bf16 = jnp.float32, jnp.bfloat16
    NQ = S // TQ

    copies = [pltpu.make_async_copy(src, dst, in_sems.at[i])
              for i, (src, dst) in enumerate((
                  (wo_hbm, wo_ref),
                  (w1t_hbm, w1t_ref), (w3t_hbm, w3t_ref), (w2_hbm, w2_ref)))]
    for cp in copies:
        cp.start()

    def out_copy(i):
        rows = pl.ds(i * TQ, TQ)
        return pltpu.make_async_copy(o_ref.at[rows], o_hbm.at[rows], out_sems.at[i])

    with jax.named_scope('phase0'):
        xn = _ln(x_ref[...].astype(f32)).astype(bf16)
        wk_in = wqkv_ref[:, D:2 * D]
        parts = []
        for t in range(DP // 128):
            lo_c, hi_c = t * G * Dh, min((t + 1) * G * Dh, D)
            parts.append(wk_in[:, lo_c:hi_c])
            parts.append(jnp.zeros((D, 128 - (hi_c - lo_c)), bf16))
        wk = jnp.concatenate(parts, axis=1)
        k_scr[...] = jnp.dot(xn, wk, preferred_element_type=f32).astype(bf16)

        tn = (((0,), (1,)), ((), ()))
        qt = jax.lax.dot_general(wqkv_ref[:, 0:D], xn, tn, preferred_element_type=f32)
        qt = qt * (Dh ** -0.5 * _LOG2E)
        vt = jax.lax.dot_general(wqkv_ref[:, 2 * D:3 * D], xn, tn,
                                 preferred_element_type=f32)
        qt_scr[...] = jnp.zeros_like(qt_scr)
        r = jax.lax.broadcasted_iota(jnp.int32, (H * VR, S), 0)
        vt_scr[...] = jnp.where(r % VR == Dh, 1.0, 0.0).astype(bf16)
        for h in range(H):
            q_lo = (h // G) * 128 + (h % G) * Dh
            qt_scr[q_lo:q_lo + Dh, :] = qt[h * Dh:(h + 1) * Dh, :].astype(bf16)
            vt_scr[h * VR:h * VR + Dh, :] = vt[h * Dh:(h + 1) * Dh, :].astype(bf16)

    for cp in copies:
        cp.wait()

    def qtile(step):
        q0 = step * TQ

        def masked_q(h):
            t = h // G
            i = h % G
            lo = pl.multiple_of(t * 128, 128)
            qt = qt_scr[pl.ds(lo, 128), q0:q0 + TQ]
            r = jax.lax.broadcasted_iota(jnp.int32, (128, TQ), 0)
            qm = jnp.where((r >= i * Dh) & (r < (i + 1) * Dh), qt, jnp.zeros_like(qt))
            return lo, qm

        def step_fn(ha, sa_ref, hb, sb_ref, mb):
            if ha is not None:
                lo, qm = masked_q(ha)
                m8 = jnp.full((8, TQ), -jnp.inf, f32)
            if hb is not None:
                v0 = pl.multiple_of(hb * VR, VR)
                acc = jnp.zeros((VR, TQ), f32)
            for c in range(S // R):
                rows = pl.ds(c * R, R)
                if ha is not None:
                    sa = jnp.dot(k_scr[rows, pl.ds(lo, 128)], qm,
                                 preferred_element_type=f32)
                    sa_ref[rows, :] = sa
                    m8 = jnp.maximum(m8, jnp.max(sa.reshape(R // 8, 8, TQ), axis=0))
                if hb is not None:
                    p = jnp.exp2(sb_ref[rows, :] - mb).astype(bf16)
                    acc = acc + jnp.dot(vt_scr[pl.ds(v0, VR), rows], p,
                                        preferred_element_type=f32)
            if hb is not None:
                l = acc[Dh:Dh + 1, :]
                ot_scr[pl.ds(v0, VR), :] = (acc / l).astype(bf16)
            if ha is not None:
                return jnp.max(m8, axis=0, keepdims=True)

        def pair(j, ma):
            h0 = 2 * j
            mb = step_fn(h0 + 1, sb_scr, h0, sa_scr, ma)
            return step_fn(h0 + 2, sa_scr, h0 + 1, sb_scr, mb)

        with jax.named_scope('attn'):
            ma = step_fn(0, sa_scr, None, None, None)
            ma = jax.lax.fori_loop(0, H // 2 - 1, pair, ma)
            mb = step_fn(H - 1, sb_scr, H - 2, sa_scr, ma)
            step_fn(None, None, H - 1, sb_scr, mb)

        with jax.named_scope('wo'):
            for h in range(H):
                otc_scr[h * Dh:(h + 1) * Dh, :] = ot_scr[h * VR:h * VR + Dh, :]
            attn = jax.lax.dot_general(otc_scr[...], wo_ref[...], (((0,), (0,)), ((), ())),
                                       preferred_element_type=f32)
        h1 = x_ref[q0:q0 + TQ, :].astype(f32) + attn

        with jax.named_scope('ffn'):
            hn = _ln(h1).astype(bf16)
            nt = (((1,), (1,)), ((), ()))
            gate = jax.lax.dot_general(hn, w1t_ref[...], nt, preferred_element_type=f32)
            up = jax.lax.dot_general(hn, w3t_ref[...], nt, preferred_element_type=f32)
            act = (gate * jax.nn.sigmoid(gate) * up).astype(bf16)
            out = jnp.dot(act, w2_ref[...], preferred_element_type=f32)
        o_ref[q0:q0 + TQ, :] = (h1 + out).astype(o_ref.dtype)
        out_copy(step).start()

    for i in range(NQ):
        qtile(i)
    for i in range(NQ):
        out_copy(i).wait()


@jax.jit
def pallas_sequential_preLN__softmax_full_mha__glu_gated_swiglu__prompt_kernel(
    A_x: jax.Array,
    A_wqkv: jax.Array,
    A_wo: jax.Array,
    B_x: jax.Array,
    B_w1: jax.Array,
    B_w3: jax.Array,
    B_w2: jax.Array,
):
    B, S, D = A_x.shape
    assert B == 1
    F = B_w1.shape[1]
    H = 32
    Dh = D // H
    G = 128 // Dh
    NT = -(-H // G)
    DP = NT * 128
    VR = 32
    TQ = 512
    R = 128
    x = A_x.reshape(S, D)
    bf16 = jnp.bfloat16

    kernel = functools.partial(_kernel, S=S, D=D, H=H, Dh=Dh, F=F, TQ=TQ, R=R)
    hbm = pl.BlockSpec(memory_space=pl.ANY)
    out = pl.pallas_call(
        kernel,
        out_shape=jax.ShapeDtypeStruct((S, D), A_x.dtype),
        in_specs=[pl.BlockSpec(memory_space=pltpu.VMEM)] * 2 + [hbm] * 4,
        out_specs=hbm,
        scratch_shapes=[
            pltpu.VMEM((D, D), bf16),
            pltpu.VMEM((F, D), bf16),
            pltpu.VMEM((F, D), bf16),
            pltpu.VMEM((F, D), bf16),
            pltpu.VMEM((S, D), bf16),
            pltpu.SemaphoreType.DMA((6,)),
            pltpu.SemaphoreType.DMA((S // TQ,)),
            pltpu.VMEM((S, DP), bf16),
            pltpu.VMEM((DP, S), bf16),
            pltpu.VMEM((H * VR, S), bf16),
            pltpu.VMEM((H * VR, TQ), bf16),
            pltpu.VMEM((D, TQ), bf16),
            pltpu.VMEM((S, TQ), jnp.float32),
            pltpu.VMEM((S, TQ), jnp.float32),
        ],
        compiler_params=pltpu.CompilerParams(
            vmem_limit_bytes=100 * 1024 * 1024,
        ),
    )(x, A_wqkv, A_wo, B_w1.T, B_w3.T, B_w2)
    return out.reshape(B, S, D)
```
